```python
import os as _os
_os.environ.setdefault("JAX_PLATFORMS", "cpu")
import jax
import jax.numpy as jnp

def _softmax(x, axis=-1):
    return jax.nn.softmax(x, axis=axis)
def _gelu(x):
    return jax.nn.gelu(x, approximate=True)
def _silu(x):
    return jax.nn.silu(x)
def _sigmoid(x):
    return jax.nn.sigmoid(x)
def _layernorm(x, axis=-1, eps=1e-5):
    m = jnp.mean(x, axis=axis, keepdims=True)
    v = jnp.var(x, axis=axis, keepdims=True)
    return (x - m) / jnp.sqrt(v + eps)
def _scatter_add(tgt, idx, src, axis=0):
    return tgt.at[idx].add(src)
def _segment_sum(src, seg, n):
    return jax.ops.segment_sum(src, seg, n)
class _Rng:
    def __init__(self, key):
        self._k = key
    def _next(self):
        self._k, sub = jax.random.split(self._k)
        return sub
    def normal(self, shape):
        return jax.random.normal(self._next(), shape, dtype=jnp.bfloat16)
    def randint(self, lo, hi, shape):
        return jax.random.randint(self._next(), shape, lo, hi, dtype=jnp.int32)
    def uniform(self, shape, lo=0.0, hi=1.0):
        return jax.random.uniform(self._next(), shape, jnp.bfloat16, lo, hi)
    def permutation(self, n):
        return jax.random.permutation(self._next(), n)


kernel_name = 'standalone__geglu_ffn__prompt'

def setup_inputs():
    _rng = _Rng(jax.random.key(int.from_bytes(__import__("os").urandom(4), "little")))
    _w = (lambda a: (lambda t: t.astype(jnp.bfloat16) if jnp.issubdtype(t.dtype, jnp.floating) else t)(jnp.asarray(a)))
    B, S, D, F = 1, 2048, 576, 4608
    return {
        "x": _w((lambda *s: _rng.normal(s) * 0.05)(B, S, D)),
        "w_gate": _w((lambda *s: _rng.normal(s) * 0.05)(D, F)),
        "w_up": _w((lambda *s: _rng.normal(s) * 0.05)(D, F)),
        "w_down": _w((lambda *s: _rng.normal(s) * 0.05)(F, D)),
    }

def reference(x, w_gate, w_up, w_down):
    return (_gelu(x @ w_gate) * (x @ w_up)) @ w_down
```

```python
import jax
import jax.numpy as jnp
import jax.experimental.pallas as pl
import jax.experimental.pallas.tpu as pltpu

_TM = 1024
_TF = 1152


def _kernel(xT_ref, wg_ref, wu_ref, wdT_ref, oT_ref, x_ref, acc_ref):
    j = pl.program_id(1)

    @pl.when(j == 0)
    def _():
        x_ref[...] = xT_ref[...].T

    x = x_ref[...]
    g = jnp.dot(x, wg_ref[...], preferred_element_type=jnp.float32)
    u = jnp.dot(x, wu_ref[...], preferred_element_type=jnp.float32)
    h = (jax.nn.gelu(g, approximate=True) * u).astype(jnp.bfloat16)
    p = jax.lax.dot_general(wdT_ref[...], h, (((1,), (1,)), ((), ())),
                            preferred_element_type=jnp.float32)

    @pl.when(j == 0)
    def _():
        acc_ref[...] = p

    @pl.when(j > 0)
    def _():
        acc_ref[...] += p

    @pl.when(j == pl.num_programs(1) - 1)
    def _():
        oT_ref[...] = acc_ref[...].astype(oT_ref.dtype)


@jax.jit
def pallas_standalone__geglu_ffn__prompt_kernel(
    x: jax.Array,
    w_gate: jax.Array,
    w_up: jax.Array,
    w_down: jax.Array,
):
    B, S, D = x.shape
    F = w_gate.shape[1]
    M = B * S
    tm, tf = _TM, _TF
    xT = x.reshape(M, D).T
    wdT = w_down.T
    outT = pl.pallas_call(
        _kernel,
        grid=(M // tm, F // tf),
        in_specs=[
            pl.BlockSpec((D, tm), lambda i, j: (0, i)),
            pl.BlockSpec((D, tf), lambda i, j: (0, j)),
            pl.BlockSpec((D, tf), lambda i, j: (0, j)),
            pl.BlockSpec((D, tf), lambda i, j: (0, j)),
        ],
        out_specs=pl.BlockSpec((D, tm), lambda i, j: (0, i)),
        out_shape=jax.ShapeDtypeStruct((D, M), x.dtype),
        scratch_shapes=[pltpu.VMEM((tm, D), jnp.bfloat16),
                        pltpu.VMEM((D, tm), jnp.float32)],
        compiler_params=pltpu.CompilerParams(
            dimension_semantics=("parallel", "arbitrary"),
            vmem_limit_bytes=100 * 1024 * 1024),
    )(xT, w_gate, w_up, wdT)
    return outT.T.reshape(B, S, D)
```

```python
import jax
import jax.numpy as jnp
import jax.experimental.pallas as pl
import jax.experimental.pallas.tpu as pltpu

_U = 128

_TF0 = 4
_DMA = (
    ("x", 0, 2), ("g", 0, 1), ("u", 0, 1),
    ("g", 1, 2), ("u", 1, 2), ("x", 2, 4),
    ("g", 2, 4), ("u", 2, 4), ("x", 4, 6),
    ("d", 0, 4), ("x", 6, 16),
)
_BLOCKS = (
    ((0,), (("T", 0, 2),)),
    ((1, 2), (("GU", 0, 1, 0, 1), ("GU", 1, 2, 0, 1))),
    ((3, 4, 5), (("T", 2, 4), ("GU", 0, 1, 1, 2), ("GU", 1, 2, 1, 2),
                 ("GU", 2, 4, 0, 2))),
    ((6, 7, 8), (("T", 4, 6), ("GU", 0, 4, 2, 4), ("GU", 4, 6, 0, 4))),
    ((9, 10), (("T", 6, 8), ("DN", 0, 4), ("GU", 6, 8, 0, 4),
               ("T", 8, 12), ("DN", 4, 8), ("GU", 8, 12, 0, 4),
               ("T", 12, 16), ("DN", 8, 12), ("GU", 12, 16, 0, 4),
               ("DN", 12, 16))),
)
_TF = 4
_GSUBS = (4, 4, 4, 4)
_DSUBS = (4, 4, 4, 2, 1, 1)


def _gate_up(x, wg, wu):
    g = jnp.dot(x, wg, preferred_element_type=jnp.float32)
    u = jnp.dot(x, wu, preferred_element_type=jnp.float32)
    return (jax.nn.gelu(g, approximate=True) * u).astype(jnp.bfloat16)


def _down(wd_t, h):
    return jax.lax.dot_general(wd_t, h, (((1,), (1,)), ((), ())),
                               preferred_element_type=jnp.float32)


def _offsets(sizes):
    out, acc = [], 0
    for s in sizes:
        out.append(acc)
        acc += s
    return out


def _make_kernel(n_it):
    tf0, tf = _TF0 * _U, _TF * _U
    gsubs = [s * _U for s in _GSUBS]
    dsubs = [s * _U for s in _DSUBS]
    goff, doff = _offsets(gsubs), _offsets(dsubs)
    nb = len(_BLOCKS)
    sem_of = {i: bi for bi, (waits, _) in enumerate(_BLOCKS) for i in waits}

    def kernel(xT_hbm, wg_hbm, wu_hbm, wdT_hbm, oT_hbm,
               xT_v, x_v, w0_v, w_v, h_v, acc_v, o_v, sem):
        w_hbm = (wg_hbm, wu_hbm, wdT_hbm)
        step = pl.program_id(0)

        def p_copy(i):
            kind, lo, hi = _DMA[i]
            sl = pl.ds(lo * _U, (hi - lo) * _U)
            s = sem.at[sem_of[i]]
            if kind == "x":
                return pltpu.make_async_copy(xT_hbm.at[:, sl], xT_v.at[:, sl], s)
            k = "gud".index(kind)
            return pltpu.make_async_copy(w_hbm[k].at[:, sl], w0_v.at[k, :, sl], s)

        def w_copy(k, f):
            off = tf0 + f * tf
            if not isinstance(f, int):
                off = pl.multiple_of(off, _U)
            return pltpu.make_async_copy(
                w_hbm[k].at[:, pl.ds(off, tf)], w_v.at[f, k], sem.at[nb + f])

        def o_copy(s):
            sl = pl.ds(doff[s], dsubs[s])
            return pltpu.make_async_copy(o_v.at[:, sl], oT_hbm.at[:, sl],
                                         sem.at[nb + n_it])

        @pl.when(step == 0)
        def _first():
            for i in range(len(_DMA)):
                p_copy(i).start()
            for f in range(n_it):
                for k in range(3):
                    w_copy(k, f).start()
            for waits, ops in _BLOCKS:
                for i in waits:
                    p_copy(i).wait()
                for op in ops:
                    sl = pl.ds(op[1] * _U, (op[2] - op[1]) * _U)
                    if op[0] == "T":
                        x_v[sl, :] = xT_v[:, sl].T
                    elif op[0] == "GU":
                        fs = pl.ds(op[3] * _U, (op[4] - op[3]) * _U)
                        h_v[sl, fs] = _gate_up(x_v[sl, :], w0_v[0, :, fs],
                                               w0_v[1, :, fs])
                    else:
                        acc_v[:, sl] = _down(w0_v[2], h_v[sl, :])

        @pl.when(step > 0)
        def _main():
            f = step - 1
            for k in range(3):
                w_copy(k, f).wait()
            for gs in range(len(gsubs)):
                h = _gate_up(x_v[pl.ds(goff[gs], gsubs[gs]), :],
                             w_v[f, 0], w_v[f, 1])
                for s in range(len(dsubs)):
                    if not goff[gs] <= doff[s] < goff[gs] + gsubs[gs]:
                        continue
                    lo = doff[s] - goff[gs]
                    dsl = pl.ds(doff[s], dsubs[s])
                    r = acc_v[:, dsl] + _down(w_v[f, 2], h[lo:lo + dsubs[s]])
                    acc_v[:, dsl] = r
                    o_v[:, dsl] = r.astype(o_v.dtype)

                    @pl.when(step == n_it)
                    def _():
                        o_copy(s).start()

        @pl.when(step == n_it)
        def _fin():
            for s in range(len(dsubs)):
                o_copy(s).wait()

    return kernel


@jax.jit
def pallas_standalone__geglu_ffn__prompt_kernel(
    x: jax.Array,
    w_gate: jax.Array,
    w_up: jax.Array,
    w_down: jax.Array,
):
    B, S, D = x.shape
    F = w_gate.shape[1]
    M = B * S
    tf0, tf = _TF0 * _U, _TF * _U
    n_it = (F - tf0) // tf
    assert tf0 + n_it * tf == F and M == sum(_GSUBS) * _U == sum(_DSUBS) * _U
    bf = jnp.bfloat16
    xT = x.reshape(M, D).T
    wdT = w_down.T
    outT = pl.pallas_call(
        _make_kernel(n_it),
        grid=(n_it + 1,),
        in_specs=[pl.BlockSpec(memory_space=pl.ANY)] * 4,
        out_specs=pl.BlockSpec(memory_space=pl.ANY),
        out_shape=jax.ShapeDtypeStruct((D, M), x.dtype),
        scratch_shapes=[
            pltpu.VMEM((D, M), bf),
            pltpu.VMEM((M, D), bf),
            pltpu.VMEM((3, D, tf0), bf),
            pltpu.VMEM((n_it, 3, D, tf), bf),
            pltpu.VMEM((M, tf0), bf),
            pltpu.VMEM((D, M), jnp.float32),
            pltpu.VMEM((D, M), x.dtype),
            pltpu.SemaphoreType.DMA((len(_BLOCKS) + n_it + 1,)),
        ],
        compiler_params=pltpu.CompilerParams(
            dimension_semantics=("arbitrary",),
            vmem_limit_bytes=100 * 1024 * 1024),
    )(xT, w_gate, w_up, wdT)
    return outT.T.reshape(B, S, D)
```

```python
import jax
import jax.numpy as jnp
import jax.experimental.pallas as pl
import jax.experimental.pallas.tpu as pltpu

_U = 128
_D = 576
_TM, _TF = 512, 1152
_NB = 3
_NSEM = 4

_FIRST = (
    ((("x", 0, 4, 0, 128),),
     (("T", 0, 4, 0, 128), ("Z", 3, 4))),
    ((("g", 0, 4, 0, 128), ("u", 0, 4, 0, 128), ("x", 0, 4, 128, 256)),
     (("T", 0, 4, 128, 256), ("PK", 0, 4, 0, 4, 0, 128, True, False))),
    ((("g", 0, 4, 128, 256), ("u", 0, 4, 128, 256), ("x", 0, 4, 256, 384)),
     (("T", 0, 4, 256, 384), ("PK", 0, 4, 0, 4, 128, 256, False, False))),
    ((("g", 0, 4, 256, 384), ("u", 0, 4, 256, 384), ("x", 0, 4, 384, _D)),
     (("T", 0, 4, 384, _D), ("PK", 0, 4, 0, 4, 256, 384, False, False))),
    ((("g", 0, 4, 384, _D), ("u", 0, 4, 384, _D)),
     (("PK", 0, 4, 0, 4, 384, _D, False, True),)),
    ((("g", 4, 9, 0, _D), ("u", 4, 9, 0, _D)),
     (("GU", 0, 2, 4, 9), ("GU", 2, 4, 4, 9))),
    ((("d", 0, 9, 0, _D), ("x", 4, 16, 0, _D)),
     (("T", 4, 8, 0, _D), ("T", 8, 12, 0, _D), ("T", 12, 16, 0, _D),
      ("DN", 0, 4))),
)
_PK_COLS = 4 * _U

_PIECES_FULL = ((0, _TM, 0, _D),)
_PIECES_LAST = ((0, 256, 0, _D), (256, 128, 0, _D),
                (384, 128, 0, 288), (384, 128, 288, 144), (384, 128, 432, 144))


def _act(g, u):
    return (jax.nn.gelu(g, approximate=True) * u).astype(jnp.bfloat16)


def _dot(a, b):
    return jnp.dot(a, b, preferred_element_type=jnp.float32)


def _down(wd_t, h):
    return jax.lax.dot_general(wd_t, h, (((1,), (1,)), ((), ())),
                               preferred_element_type=jnp.float32)


def _make_kernel(nmg, nfc, n_it):
    ng = len(_FIRST)
    units_per_mg = _TM // _U
    final = [(b % nmg, (b - 1) // _NB + 1, (b - 1) % _NB)
             for b in range(nmg * (nfc - 1), nmg * nfc)]

    def pieces(j):
        return _PIECES_LAST if j == _NB - 1 else _PIECES_FULL

    def kernel(xT_hbm, wg_hbm, wu_hbm, wdT_hbm, oT_hbm,
               xT_v, x_v, w_v, h_v, acc_v, o_v, gu_v, sem):
        w_hbm = (wg_hbm, wu_hbm, wdT_hbm)
        step = pl.program_id(0)

        def group(gi):
            s = sem.at[gi % _NSEM]
            cps = []
            if gi < ng:
                for kind, lo, hi, rlo, rhi in _FIRST[gi][0]:
                    cs = pl.ds(lo * _U, (hi - lo) * _U)
                    rs = pl.ds(rlo, rhi - rlo)
                    if kind == "x":
                        cps.append(pltpu.make_async_copy(
                            xT_hbm.at[rs, cs], xT_v.at[rs, cs], s))
                    else:
                        k = "gud".index(kind)
                        cps.append(pltpu.make_async_copy(
                            w_hbm[k].at[rs, cs], w_v.at[0, k, rs, cs], s))
            else:
                for fc in range(1, nfc):
                    for k in range(3):
                        cps.append(pltpu.make_async_copy(
                            w_hbm[k].at[:, pl.ds(fc * _TF, _TF)],
                            w_v.at[fc, k], s))
            return cps

        def o_copy(mg, lo, sz, rlo, rsz):
            rs = pl.ds(rlo, rsz)
            return pltpu.make_async_copy(
                o_v.at[mg, rs, pl.ds(lo, sz)],
                oT_hbm.at[rs, pl.ds(mg * _TM + lo, sz)],
                sem.at[(ng + 1) % _NSEM])

        @pl.when(step == 0)
        def _first():
            for gi in range(_NSEM):
                for c in group(gi):
                    c.start()
            acc_v[1:3] = jnp.zeros((2,) + acc_v.shape[1:], jnp.float32)

            for gi, (_, ops) in enumerate(_FIRST):
                for c in group(gi):
                    c.wait()
                if gi + _NSEM <= ng:
                    for c in group(gi + _NSEM):
                        c.start()
                for op in ops:
                    if op[0] == "Z":
                        acc_v[op[1]:op[2]] = jnp.zeros(
                            (op[2] - op[1],) + acc_v.shape[1:], jnp.float32)
                        continue
                    mg = op[1] // units_per_mg
                    n = (op[2] - op[1]) * _U
                    sl = pl.ds(op[1] * _U - mg * _TM, n)
                    if op[0] == "T":
                        ks = pl.ds(op[3], op[4] - op[3])
                        x_v[mg, sl, ks] = xT_v[ks, pl.ds(op[1] * _U, n)].T
                    elif op[0] == "DN":
                        acc_v[mg, :, sl] = _down(w_v[0, 2], h_v[sl, :])
                    elif op[0] == "GU":
                        fs = pl.ds(op[3] * _U, (op[4] - op[3]) * _U)
                        x = x_v[mg, sl, :]
                        h_v[sl, fs] = _act(_dot(x, w_v[0, 0, :, fs]),
                                           _dot(x, w_v[0, 1, :, fs]))
                    else:
                        fs = pl.ds(op[3] * _U, (op[4] - op[3]) * _U)
                        ks = pl.ds(op[5], op[6] - op[5])
                        x = x_v[mg, sl, ks]
                        g = _dot(x, w_v[0, 0, ks, fs])
                        u = _dot(x, w_v[0, 1, ks, fs])
                        if not op[7]:
                            g = g + gu_v[0, sl, fs]
                            u = u + gu_v[1, sl, fs]
                        if op[8]:
                            h_v[sl, fs] = _act(g, u)
                        else:
                            gu_v[0, sl, fs] = g
                            gu_v[1, sl, fs] = u

        @pl.when(step > 0)
        def _main():
            @pl.when(step == 2)
            def _():
                for c in group(ng):
                    c.wait()

            for j in range(_NB):
                b = step * _NB + (1 + j - _NB)
                mg = jnp.bitwise_and(b, nmg - 1)
                fc = jax.lax.shift_right_logical(b, 2)
                x = x_v[mg]
                h = _act(_dot(x, w_v[fc, 0]), _dot(x, w_v[fc, 1]))
                for lo, sz, rlo, rsz in pieces(j):
                    cs, rs = pl.ds(lo, sz), pl.ds(rlo, rsz)
                    r = acc_v[mg, rs, cs] + _down(w_v[fc, 2, rs, :],
                                                  h[lo:lo + sz])
                    acc_v[mg, rs, cs] = r
                    o_v[mg, rs, cs] = r.astype(o_v.dtype)
                    for fmg, fstep, fj in final:
                        if fj == j:
                            @pl.when(step == fstep)
                            def _():
                                o_copy(fmg, lo, sz, rlo, rsz).start()

        @pl.when(step == n_it)
        def _fin():
            for fmg, _, fj in final:
                for pc in pieces(fj):
                    o_copy(fmg, *pc).wait()

    return kernel


@jax.jit
def pallas_standalone__geglu_ffn__prompt_kernel(
    x: jax.Array,
    w_gate: jax.Array,
    w_up: jax.Array,
    w_down: jax.Array,
):
    B, S, D = x.shape
    F = w_gate.shape[1]
    M = B * S
    nmg, nfc = M // _TM, F // _TF
    assert D == _D and nmg == 4 and nmg * _TM == M and nfc * _TF == F
    n_it = (nmg * nfc - 1) // _NB
    assert 1 + n_it * _NB == nmg * nfc
    bf = jnp.bfloat16
    xT = x.reshape(M, D).T
    wdT = w_down.T
    outT = pl.pallas_call(
        _make_kernel(nmg, nfc, n_it),
        grid=(n_it + 1,),
        in_specs=[pl.BlockSpec(memory_space=pl.ANY)] * 4,
        out_specs=pl.BlockSpec(memory_space=pl.ANY),
        out_shape=jax.ShapeDtypeStruct((D, M), x.dtype),
        scratch_shapes=[
            pltpu.VMEM((D, M), bf),
            pltpu.VMEM((nmg, _TM, D), bf),
            pltpu.VMEM((nfc, 3, D, _TF), bf),
            pltpu.VMEM((_TM, _TF), bf),
            pltpu.VMEM((nmg, D, _TM), jnp.float32),
            pltpu.VMEM((nmg, D, _TM), x.dtype),
            pltpu.VMEM((2, _TM, _PK_COLS), jnp.float32),
            pltpu.SemaphoreType.DMA((_NSEM,)),
        ],
        compiler_params=pltpu.CompilerParams(
            dimension_semantics=("arbitrary",),
            vmem_limit_bytes=100 * 1024 * 1024),
    )(xT, w_gate, w_up, wdT)
    return outT.T.reshape(B, S, D)
```

```python
import jax
import jax.numpy as jnp
import jax.experimental.pallas as pl
import jax.experimental.pallas.tpu as pltpu

_U = 128
_D = 576
_TM, _TF = 512, 1152
_NB = 3
_NSEM = 4

_FIRST = (
    ((("x", 0, 4, 512, _D),),
     (("T", 0, 4, 512, _D),)),
    ((("g", 0, 4, 512, _D), ("u", 0, 4, 512, _D)),
     (("PK", 0, 4, 0, 4, 512, _D, True, False),)),
    ((("g", 4, 8, 512, _D), ("u", 4, 8, 512, _D), ("x", 0, 4, 0, 256),
      ("g", 0, 4, 0, 128), ("u", 0, 4, 0, 128)),
     (("T", 0, 4, 0, 128), ("T", 0, 4, 128, 256),
      ("PK", 0, 4, 4, 8, 512, _D, True, False),
      ("PK", 0, 4, 0, 4, 0, 128, False, False))),
    ((("g", 0, 4, 128, 384), ("u", 0, 4, 128, 384), ("x", 0, 4, 256, 512),
      ("g", 0, 4, 384, 512), ("u", 0, 4, 384, 512)),
     (("T", 0, 4, 256, 384), ("T", 0, 4, 384, 512),
      ("PK", 0, 4, 0, 4, 128, 256, False, False),
      ("PK", 0, 4, 0, 4, 256, 512, False, True))),
    ((("g", 4, 8, 0, 512), ("u", 4, 8, 0, 512),
      ("g", 8, 9, 0, _D), ("u", 8, 9, 0, _D)),
     (("PK", 0, 4, 4, 8, 0, 512, False, True),
      ("GU", 0, 2, 8, 9), ("GU", 2, 4, 8, 9))),
    ((("d", 0, 9, 0, _D), ("x", 4, 16, 0, _D)),
     (("T", 4, 8, 0, _D), ("T", 8, 12, 0, _D), ("T", 12, 16, 0, _D),
      ("DN", 0, 4), ("Z", 3, 4))),
)
_PK_COLS = 8 * _U

_PIECES_FULL = ((0, _TM, 0, _D),)
_PIECES_LAST = ((0, 256, 0, _D), (256, 128, 0, _D),
                (384, 128, 0, 288), (384, 128, 288, 144), (384, 128, 432, 144))


def _act(g, u):
    return (jax.nn.gelu(g, approximate=True) * u).astype(jnp.bfloat16)


def _dot(a, b):
    return jnp.dot(a, b, preferred_element_type=jnp.float32)


def _down(wd_t, h):
    return jax.lax.dot_general(wd_t, h, (((1,), (1,)), ((), ())),
                               preferred_element_type=jnp.float32)


def _make_kernel(nmg, nfc, n_it):
    ng = len(_FIRST)
    units_per_mg = _TM // _U
    final = [(b % nmg, (b - 1) // _NB + 1, (b - 1) % _NB)
             for b in range(nmg * (nfc - 1), nmg * nfc)]

    def pieces(j):
        return _PIECES_LAST if j == _NB - 1 else _PIECES_FULL

    def kernel(xT_hbm, wg_hbm, wu_hbm, wdT_hbm, oT_hbm,
               xT_v, x_v, w_v, h_v, acc_v, o_v, gu_v, sem):
        w_hbm = (wg_hbm, wu_hbm, wdT_hbm)
        step = pl.program_id(0)

        def group(gi):
            s = sem.at[gi % _NSEM]
            cps = []
            if gi < ng:
                for kind, lo, hi, rlo, rhi in _FIRST[gi][0]:
                    cs = pl.ds(lo * _U, (hi - lo) * _U)
                    rs = pl.ds(rlo, rhi - rlo)
                    if kind == "x":
                        cps.append(pltpu.make_async_copy(
                            xT_hbm.at[rs, cs], xT_v.at[rs, cs], s))
                    else:
                        k = "gud".index(kind)
                        cps.append(pltpu.make_async_copy(
                            w_hbm[k].at[rs, cs], w_v.at[0, k, rs, cs], s))
            else:
                for fc in range(1, nfc):
                    for k in range(3):
                        cps.append(pltpu.make_async_copy(
                            w_hbm[k].at[:, pl.ds(fc * _TF, _TF)],
                            w_v.at[fc, k], s))
            return cps

        def o_copy(mg, lo, sz, rlo, rsz):
            rs = pl.ds(rlo, rsz)
            return pltpu.make_async_copy(
                o_v.at[mg, rs, pl.ds(lo, sz)],
                oT_hbm.at[rs, pl.ds(mg * _TM + lo, sz)],
                sem.at[(ng + 1) % _NSEM])

        @pl.when(step == 0)
        def _first():
            for gi in range(_NSEM):
                for c in group(gi):
                    c.start()
            acc_v[1:3] = jnp.zeros((2,) + acc_v.shape[1:], jnp.float32)

            for gi, (_, ops) in enumerate(_FIRST):
                for c in group(gi):
                    c.wait()
                if gi + _NSEM <= ng:
                    for c in group(gi + _NSEM):
                        c.start()
                for op in ops:
                    if op[0] == "Z":
                        acc_v[op[1]:op[2]] = jnp.zeros(
                            (op[2] - op[1],) + acc_v.shape[1:], jnp.float32)
                        continue
                    mg = op[1] // units_per_mg
                    n = (op[2] - op[1]) * _U
                    sl = pl.ds(op[1] * _U - mg * _TM, n)
                    if op[0] == "T":
                        ks = pl.ds(op[3], op[4] - op[3])
                        x_v[mg, sl, ks] = xT_v[ks, pl.ds(op[1] * _U, n)].T
                    elif op[0] == "DN":
                        acc_v[mg, :, sl] = _down(w_v[0, 2], h_v[sl, :])
                    elif op[0] == "GU":
                        fs = pl.ds(op[3] * _U, (op[4] - op[3]) * _U)
                        x = x_v[mg, sl, :]
                        h_v[sl, fs] = _act(_dot(x, w_v[0, 0, :, fs]),
                                           _dot(x, w_v[0, 1, :, fs]))
                    else:
                        fs = pl.ds(op[3] * _U, (op[4] - op[3]) * _U)
                        ks = pl.ds(op[5], op[6] - op[5])
                        x = x_v[mg, sl, ks]
                        g = _dot(x, w_v[0, 0, ks, fs])
                        u = _dot(x, w_v[0, 1, ks, fs])
                        if not op[7]:
                            g = g + gu_v[0, sl, fs]
                            u = u + gu_v[1, sl, fs]
                        if op[8]:
                            h_v[sl, fs] = _act(g, u)
                        else:
                            gu_v[0, sl, fs] = g
                            gu_v[1, sl, fs] = u

        @pl.when(step > 0)
        def _main():
            @pl.when(step == 2)
            def _():
                for c in group(ng):
                    c.wait()

            for j in range(_NB):
                b = step * _NB + (1 + j - _NB)
                mg = jnp.bitwise_and(b, nmg - 1)
                fc = jax.lax.shift_right_logical(b, 2)
                x = x_v[mg]
                h = _act(_dot(x, w_v[fc, 0]), _dot(x, w_v[fc, 1]))
                for lo, sz, rlo, rsz in pieces(j):
                    cs, rs = pl.ds(lo, sz), pl.ds(rlo, rsz)
                    r = acc_v[mg, rs, cs] + _down(w_v[fc, 2, rs, :],
                                                  h[lo:lo + sz])
                    acc_v[mg, rs, cs] = r
                    o_v[mg, rs, cs] = r.astype(o_v.dtype)
                    for fmg, fstep, fj in final:
                        if fj == j:
                            @pl.when(step == fstep)
                            def _():
                                o_copy(fmg, lo, sz, rlo, rsz).start()

        @pl.when(step == n_it)
        def _fin():
            for fmg, _, fj in final:
                for pc in pieces(fj):
                    o_copy(fmg, *pc).wait()

    return kernel


@jax.jit
def pallas_standalone__geglu_ffn__prompt_kernel(
    x: jax.Array,
    w_gate: jax.Array,
    w_up: jax.Array,
    w_down: jax.Array,
):
    B, S, D = x.shape
    F = w_gate.shape[1]
    M = B * S
    nmg, nfc = M // _TM, F // _TF
    assert D == _D and nmg == 4 and nmg * _TM == M and nfc * _TF == F
    n_it = (nmg * nfc - 1) // _NB
    assert 1 + n_it * _NB == nmg * nfc
    bf = jnp.bfloat16
    xT = x.reshape(M, D).T
    wdT = w_down.T
    outT = pl.pallas_call(
        _make_kernel(nmg, nfc, n_it),
        grid=(n_it + 1,),
        in_specs=[pl.BlockSpec(memory_space=pl.ANY)] * 4,
        out_specs=pl.BlockSpec(memory_space=pl.ANY),
        out_shape=jax.ShapeDtypeStruct((D, M), x.dtype),
        scratch_shapes=[
            pltpu.VMEM((D, M), bf),
            pltpu.VMEM((nmg, _TM, D), bf),
            pltpu.VMEM((nfc, 3, D, _TF), bf),
            pltpu.VMEM((_TM, _TF), bf),
            pltpu.VMEM((nmg, D, _TM), jnp.float32),
            pltpu.VMEM((nmg, D, _TM), x.dtype),
            pltpu.VMEM((2, _TM, _PK_COLS), jnp.float32),
            pltpu.SemaphoreType.DMA((_NSEM,)),
        ],
        compiler_params=pltpu.CompilerParams(
            dimension_semantics=("arbitrary",),
            vmem_limit_bytes=100 * 1024 * 1024),
    )(xT, w_gate, w_up, wdT)
    return outT.T.reshape(B, S, D)
```

```python
import jax
import jax.numpy as jnp
import jax.experimental.pallas as pl
import jax.experimental.pallas.tpu as pltpu

_U = 128
_D = 576
_KM, _KR = 512, 64
_TF = 512
_NSEM = 4

_FIRST = (
    ((("x", 0, 4, _KM, _D),),
     (("T", 0, 4, _KM, _D),)),
    ((("g", _KM, _D), ("u", _KM, _D), ("x", 4, 8, _KM, _D)),
     (("T", 4, 8, _KM, _D),
      ("PK", 0, 4, _KM, _D, True, False), ("PK", 4, 6, _KM, _D, True, False))),
    ((("x", 8, 16, _KM, _D), ("r",), ("x", 0, 4, 0, 256)),
     (("T", 8, 12, _KM, _D), ("T", 12, 16, _KM, _D), ("T", 0, 4, 0, 256),
      ("WS",), ("XR",),
      ("PK", 6, 8, _KM, _D, True, False), ("PK", 8, 12, _KM, _D, True, False),
      ("PK", 12, 16, _KM, _D, True, False), ("R1",))),
    ((("g", 0, _KM), ("u", 0, _KM), ("x", 0, 4, 256, _KM), ("x", 4, 8, 0, _KM)),
     (("T", 0, 4, 256, _KM), ("T", 4, 8, 0, _KM),
      ("PK", 0, 4, 0, 256, False, False), ("PK", 0, 4, 256, _KM, False, True),
      ("PK", 4, 8, 0, _KM, False, True))),
    ((("x", 8, 16, 0, _KM), ("d", 0, _D)),
     (("T", 8, 12, 0, _KM), ("T", 12, 16, 0, _KM),
      ("DN", 0, 4), ("PK", 8, 12, 0, _KM, False, True),
      ("DN", 4, 8), ("PK", 12, 16, 0, _KM, False, True),
      ("DN", 8, 12), ("DN", 12, 16))),
)

_TM = 512
_PIECES = (
    ((0, 512, 0, _D),),
    ((512, 512, 0, _D),),
    ((1024, 512, 0, _D),),
    ((1536, 256, 0, _D), (1792, 256, 0, 288), (1792, 256, 288, 288)),
)

_F32, _BF16 = jnp.float32, jnp.bfloat16


def _act(g, u):
    return (jax.nn.gelu(g, approximate=True) * u).astype(_BF16)


def _dot(a, b):
    return jnp.dot(a, b, preferred_element_type=_F32)


def _down(wd_t, h):
    return jax.lax.dot_general(wd_t, h, (((1,), (1,)), ((), ())),
                               preferred_element_type=_F32)


def _make_kernel(n_it, nmt):
    ng = len(_FIRST)
    tf, nc = _TF, _U

    def kernel(xT_hbm, wg_hbm, wu_hbm, wdT_hbm, oT_hbm,
               xT_v, x_v, w_v, h_v, acc_v, o_v, gu_v,
               wr_v, wf_v, xr_v, rt_v, r_v, ws_s, sem, sem_ws):
        w_hbm = (wg_hbm, wu_hbm, wdT_hbm)
        step = pl.program_id(0)

        def group(gi):
            s = sem.at[gi % _NSEM]
            cps = []
            if gi < ng:
                for ent in _FIRST[gi][0]:
                    if ent[0] == "r":
                        for i in range(n_it):
                            cps.append(pltpu.make_async_copy(
                                wu_hbm.at[pl.ds(_KM, _KR),
                                          pl.ds((i + 2) * tf - nc, nc)],
                                wr_v.at[i], s))
                    elif ent[0] == "x":
                        _, lo, hi, klo, khi = ent
                        rs = pl.ds(klo, khi - klo)
                        cs = pl.ds(lo * _U, (hi - lo) * _U)
                        cps.append(pltpu.make_async_copy(
                            xT_hbm.at[rs, cs], xT_v.at[rs, cs], s))
                    else:
                        k = "gud".index(ent[0])
                        rs = pl.ds(ent[1], ent[2] - ent[1])
                        cps.append(pltpu.make_async_copy(
                            w_hbm[k].at[rs, pl.ds(0, tf)], w_v.at[0, k, rs], s))
            else:
                for fc in (range(1, 2) if gi == ng else range(2, n_it + 1)):
                    for k in range(3):
                        cps.append(pltpu.make_async_copy(
                            w_hbm[k].at[:, pl.ds(fc * tf, tf)],
                            w_v.at[fc, k], s))
            return cps

        def ws_copy():
            return pltpu.make_async_copy(wf_v, ws_s, sem_ws.at[0])

        def o_copy(lo, sz, rlo, rsz):
            rs, cs = pl.ds(rlo, rsz), pl.ds(lo, sz)
            return pltpu.make_async_copy(o_v.at[rs, cs], oT_hbm.at[rs, cs],
                                         sem.at[(ng + 2) % _NSEM])

        @pl.when(step == 0)
        def _first():
            for gi in range(_NSEM):
                for c in group(gi):
                    c.start()
            for gi, (_, ops) in enumerate(_FIRST):
                for c in group(gi):
                    c.wait()
                if gi + _NSEM <= ng + 1:
                    for c in group(gi + _NSEM):
                        c.start()
                for op in ops:
                    if op[0] == "WS":
                        for i in range(1, n_it):
                            wf_v[(i - 1) * nc:i * nc, :] = (
                                wr_v[i].astype(_F32).T)
                        ws_copy().start()
                        continue
                    if op[0] == "XR":
                        for mt in range(nmt):
                            xr_v[mt // 8, pl.ds(mt % 8, _KR, stride=8), :] = (
                                xT_v[_KM:_D, mt * _U:(mt + 1) * _U]
                                .astype(_F32))
                        continue
                    if op[0] == "R1":
                        for q in range(len(_PIECES)):
                            rows = pl.ds(q * _TM, _TM)
                            r_v[rows, :] = _dot(x_v[rows, _KM:_D], wr_v[0])
                        continue
                    sl = pl.ds(op[1] * _U, (op[2] - op[1]) * _U)
                    if op[0] == "T":
                        ks = pl.ds(op[3], op[4] - op[3])
                        x_v[sl, ks] = xT_v[ks, sl].T
                    elif op[0] == "DN":
                        acc_v[:, sl] = _down(w_v[0, 2], h_v[sl, :])
                    else:
                        ks = pl.ds(op[3], op[4] - op[3])
                        x = x_v[sl, ks]
                        g = _dot(x, w_v[0, 0, ks, :])
                        u = _dot(x, w_v[0, 1, ks, :])
                        if not op[5]:
                            g = g + gu_v[0, sl, :]
                            u = u + gu_v[1, sl, :]
                        if op[6]:
                            h_v[sl, :] = _act(g, u)
                        else:
                            gu_v[0, sl, :] = g
                            gu_v[1, sl, :] = u
            for c in group(ng):
                c.wait()
            ws_copy().wait()

        @pl.when(step > 0)
        def _main():
            @pl.when(step == 2)
            def _():
                for c in group(ng + 1):
                    c.wait()

            no8 = jnp.full((8, _U), step, jnp.int32) < 0
            no8b = jnp.full((8, _U), step, jnp.int32) < -1
            no16 = jnp.full((16, _U), step, jnp.int32) < 0

            base = jnp.minimum(step - 1, n_it - 2) * nc

            def column(n, carry):
                row = base + n
                wv = jnp.full((8, _U), ws_s[row, 0], _F32)
                wv = jnp.where(no8, carry[0], jnp.where(no8b, carry[1], wv))
                a = wv * xr_v[0, 0:8, :]
                b = wv * xr_v[1, 0:8, :]
                for k in range(1, _KR):
                    wv = jnp.full((8, _U), ws_s[row, k], _F32)
                    a = a + wv * xr_v[0, k * 8:k * 8 + 8, :]
                    b = b + wv * xr_v[1, k * 8:k * 8 + 8, :]
                rs = pl.ds(pl.multiple_of(n * 8, 8), 8)
                rt_v[0, rs, :] = a
                rt_v[1, rs, :] = b
                return a, b

            zero = jnp.zeros((8, _U), _F32)
            jax.lax.fori_loop(0, nc, column, (zero, zero), unroll=True)
            r_next = [rt_v[mt // 8, pl.ds(mt % 8, nc, stride=8), :].T
                      for mt in range(nmt)]

            for q, pieces in enumerate(_PIECES):
                sl = pl.ds(q * _TM, _TM)
                x = x_v[sl, :]
                g = _dot(x, w_v[step, 0])
                u1 = _dot(x, w_v[step, 1, :, 0:tf - nc])
                u2 = (_dot(x[:, 0:_KM], w_v[step, 1, 0:_KM, tf - nc:tf])
                      + r_v[sl, :])
                h = jnp.concatenate([_act(g[:, 0:tf - nc], u1),
                                     _act(g[:, tf - nc:tf], u2)], axis=1)
                for pi, (lo, sz, rlo, rsz) in enumerate(pieces):
                    cs, rs = pl.ds(lo, sz), pl.ds(rlo, rsz)
                    wd = w_v[step, 2, rs, :]
                    if q == len(_PIECES) - 1 and pi == 0:
                        ta, tb = r_next[0][nc - 8:], r_next[1][nc - 8:]
                        for mt in range(2, nmt, 2):
                            ta = ta + r_next[mt][nc - 8:]
                            tb = tb + r_next[mt + 1][nc - 8:]
                        t = jnp.concatenate([ta, tb], axis=0).astype(_BF16)
                        w00 = jnp.where(no16, t, wd[0:16, 0:_U])
                        top = jnp.concatenate([w00, wd[0:16, _U:]], axis=1)
                        wd = jnp.concatenate([top, wd[16:]], axis=0)
                    l0 = lo - q * _TM
                    r = acc_v[rs, cs] + _down(wd, h[l0:l0 + sz])
                    acc_v[rs, cs] = r
                    o_v[rs, cs] = r.astype(o_v.dtype)

                    @pl.when(step == n_it)
                    def _():
                        o_copy(lo, sz, rlo, rsz).start()

            for mt in range(nmt):
                r_v[mt * _U:(mt + 1) * _U, :] = r_next[mt]

        @pl.when(step == n_it)
        def _fin():
            for pieces in _PIECES:
                for pc in pieces:
                    o_copy(*pc).wait()

    return kernel


@jax.jit
def pallas_standalone__geglu_ffn__prompt_kernel(
    x: jax.Array,
    w_gate: jax.Array,
    w_up: jax.Array,
    w_down: jax.Array,
):
    B, S, D = x.shape
    F = w_gate.shape[1]
    M = B * S
    n_it = F // _TF - 1
    nmt = M // _U
    assert D == _D and nmt == 16 and (n_it + 1) * _TF == F
    assert M == len(_PIECES) * _TM
    xT = x.reshape(M, D).T
    wdT = w_down.T
    outT = pl.pallas_call(
        _make_kernel(n_it, nmt),
        grid=(n_it + 1,),
        in_specs=[pl.BlockSpec(memory_space=pl.ANY)] * 4,
        out_specs=pl.BlockSpec(memory_space=pl.ANY),
        out_shape=jax.ShapeDtypeStruct((D, M), x.dtype),
        scratch_shapes=[
            pltpu.VMEM((D, M), _BF16),
            pltpu.VMEM((M, D), _BF16),
            pltpu.VMEM((n_it + 1, 3, D, _TF), _BF16),
            pltpu.VMEM((M, _TF), _BF16),
            pltpu.VMEM((D, M), _F32),
            pltpu.VMEM((D, M), x.dtype),
            pltpu.VMEM((2, M, _TF), _F32),
            pltpu.VMEM((n_it, _KR, _U), _BF16),
            pltpu.VMEM(((n_it - 1) * _U, _KR), _F32),
            pltpu.VMEM((2, _KR * 8, _U), _F32),
            pltpu.VMEM((2, _U * 8, _U), _F32),
            pltpu.VMEM((M, _U), _F32),
            pltpu.SMEM(((n_it - 1) * _U, _KR), _F32),
            pltpu.SemaphoreType.DMA((_NSEM,)),
            pltpu.SemaphoreType.DMA((1,)),
        ],
        compiler_params=pltpu.CompilerParams(
            dimension_semantics=("arbitrary",),
            vmem_limit_bytes=100 * 1024 * 1024),
    )(xT, w_gate, w_up, wdT)
    return outT.T.reshape(B, S, D)
```

```python
import jax
import jax.numpy as jnp
import jax.experimental.pallas as pl
import jax.experimental.pallas.tpu as pltpu

_U = 128
_D = 576
_KM, _KR = 512, 64
_CT = 3
_TF = _CT * _U
_TM = 512
_NSEM = 4
_NE = 13
_EXTRA = ((0, _CT - 1), (1, _CT - 2))

_FIRST = (
    ((("x", 0, 4, _KM, _D),),
     (("T", 0, 4, _KM, _D),)),
    ((("g", _KM, _D), ("u", _KM, _D), ("x", 4, 8, _KM, _D)),
     (("T", 4, 8, _KM, _D),
      ("PK", 0, 2, _KM, _D, True, False), ("PK", 2, 4, _KM, _D, True, False),
      ("PK", 4, 6, _KM, _D, True, False), ("PK", 6, 8, _KM, _D, True, False))),
    ((("r0",), ("x", 8, 16, _KM, _D), ("x", 0, 4, 0, 256)),
     (("T", 8, 12, _KM, _D), ("T", 12, 16, _KM, _D), ("T", 0, 4, 0, 256),
      ("XR",), ("R1", 0, 8),
      ("PK", 8, 12, _KM, _D, True, False), ("PK", 12, 16, _KM, _D, True, False),
      ("R1", 8, 16))),
    ((("g", 0, _KM), ("u", 0, _KM), ("x", 0, 4, 256, _KM), ("x", 4, 8, 0, 256),
      ("rr",)),
     (("WS",), ("T", 0, 4, 256, _KM), ("T", 4, 8, 0, 256),
      ("PK", 0, 4, 0, 256, False, False), ("PK", 0, 4, 256, _KM, False, True),
      ("PK", 4, 8, 0, 256, False, False))),
    ((("x", 4, 8, 256, _KM), ("x", 8, 16, 0, _KM), ("d", 0, _D)),
     (("T", 4, 8, 256, _KM), ("T", 8, 12, 0, _KM), ("T", 12, 16, 0, _KM),
      ("DN", 0, 4), ("PK", 4, 8, 256, _KM, False, True),
      ("PK", 8, 12, 0, _KM, False, True), ("DN", 4, 8),
      ("PK", 12, 16, 0, _KM, False, True), ("DN", 8, 12), ("DN", 12, 16))),
)

_LAST = (
    (0, 512, ((0, _D),)),
    (512, 512, ((0, _D),)),
    (1024, 512, ((0, _D),)),
    (1536, 256, ((0, _D),)),
    (1792, 128, ((0, _D),)),
    (1920, 128, ((0, 288), (288, 288))),
)

_F32, _BF16 = jnp.float32, jnp.bfloat16


def _act(g, u):
    return (jax.nn.gelu(g, approximate=True) * u).astype(_BF16)


def _dot(a, b):
    return jnp.dot(a, b, preferred_element_type=_F32)


def _down(wd_t, h):
    return jax.lax.dot_general(wd_t, h, (((1,), (1,)), ((), ())),
                               preferred_element_type=_F32)


def _make_kernel(nch, nmt):
    ng = len(_FIRST)
    tf, nc = _TF, _U
    last = nch - 1
    hc = nc // 2
    vtiles = [(m, last * tf + ct * nc) for m, ct in _EXTRA]
    vtiles += [(1, (c + 1) * tf - nc) for c in range(2, nch)]
    assert (nch - 2) * _NE >= len(_EXTRA) * hc

    def kernel(xT_hbm, wg_hbm, wu_hbm, wdT_hbm, oT_hbm,
               xT_v, x_v, w_v, h_v, acc_v, o_v, gu_v,
               wr0_v, wr_v, wf_v, xr_v, rt_v, r_v, rt2_v, ws_s, sem, sem_ws):
        w_hbm = (wg_hbm, wu_hbm, wdT_hbm)
        step = pl.program_id(0)

        def group(gi):
            s = sem.at[gi % _NSEM]
            rem = pl.ds(_KM, _KR)
            cps = []
            if gi < ng:
                for ent in _FIRST[gi][0]:
                    if ent[0] == "r0":
                        cps.append(pltpu.make_async_copy(
                            wu_hbm.at[rem, pl.ds(2 * tf - nc, nc)], wr0_v, s))
                    elif ent[0] == "rr":
                        for i, (m, col) in enumerate(vtiles):
                            cps.append(pltpu.make_async_copy(
                                w_hbm[m].at[rem, pl.ds(col, nc)],
                                wr_v.at[i], s))
                    elif ent[0] == "x":
                        _, lo, hi, klo, khi = ent
                        rs = pl.ds(klo, khi - klo)
                        cs = pl.ds(lo * _U, (hi - lo) * _U)
                        cps.append(pltpu.make_async_copy(
                            xT_hbm.at[rs, cs], xT_v.at[rs, cs], s))
                    else:
                        k = "gud".index(ent[0])
                        rs = pl.ds(ent[1], ent[2] - ent[1])
                        cps.append(pltpu.make_async_copy(
                            w_hbm[k].at[rs, pl.ds(0, tf)], w_v.at[0, k, rs], s))
            else:
                for c in (range(1, 2) if gi == ng else range(2, nch)):
                    for k in range(3):
                        cps.append(pltpu.make_async_copy(
                            w_hbm[k].at[:, pl.ds(c * tf, tf)], w_v.at[c, k], s))
            return cps

        def ws_copy():
            return pltpu.make_async_copy(wf_v, ws_s, sem_ws.at[0])

        def o_copy(lo, sz, rlo, rsz):
            rs, cs = pl.ds(rlo, rsz), pl.ds(lo, sz)
            return pltpu.make_async_copy(o_v.at[rs, cs], oT_hbm.at[rs, cs],
                                         sem.at[(ng + 2) % _NSEM])

        @pl.when(step == 0)
        def _first():
            for gi in range(_NSEM):
                for c in group(gi):
                    c.start()
            for gi, (_, ops) in enumerate(_FIRST):
                for c in group(gi):
                    c.wait()
                if gi + _NSEM <= ng + 1:
                    for c in group(gi + _NSEM):
                        c.start()
                for op in ops:
                    if op[0] == "WS":
                        for i in range(len(vtiles)):
                            wt = wr_v[i].astype(_F32).T
                            wf_v[i * hc:(i + 1) * hc, :] = jnp.concatenate(
                                [wt[:hc], wt[hc:]], axis=1)
                        ws_copy().start()
                        continue
                    if op[0] == "XR":
                        for mt in range(nmt):
                            xr_v[mt // 8, pl.ds(mt % 8, _KR, stride=8), :] = (
                                xT_v[_KM:_D, mt * _U:(mt + 1) * _U]
                                .astype(_F32))
                        continue
                    if op[0] == "R1":
                        for q in range(op[1] // 2, op[2] // 2):
                            rows = pl.ds(q * 2 * _U, 2 * _U)
                            r_v[rows, :] = _dot(x_v[rows, _KM:_D], wr0_v[...])
                        continue
                    sl = pl.ds(op[1] * _U, (op[2] - op[1]) * _U)
                    if op[0] == "T":
                        ks = pl.ds(op[3], op[4] - op[3])
                        x_v[sl, ks] = xT_v[ks, sl].T
                    elif op[0] == "DN":
                        acc_v[:, sl] = _down(w_v[0, 2], h_v[sl, :])
                    else:
                        ks = pl.ds(op[3], op[4] - op[3])
                        x = x_v[sl, ks]
                        g = _dot(x, w_v[0, 0, ks, :])
                        u = _dot(x, w_v[0, 1, ks, :])
                        if not op[5]:
                            g = g + gu_v[0, sl, :]
                            u = u + gu_v[1, sl, :]
                        if op[6]:
                            h_v[sl, :] = _act(g, u)
                        else:
                            gu_v[0, sl, :] = g
                            gu_v[1, sl, :] = u
            for c in group(ng):
                c.wait()
            ws_copy().wait()

        @pl.when(jnp.logical_and(step > 0, step < last))
        def _middle():
            @pl.when(step == 2)
            def _():
                for c in group(ng + 1):
                    c.wait()

            no8 = jnp.full((8, _U), step, jnp.int32) < 0
            no8b = jnp.full((8, _U), step, jnp.int32) < -1
            no16 = jnp.full((16, _U), step, jnp.int32) < 0

            def column(row, col, dst, drow, carry):
                wv = jnp.full((8, _U), ws_s[row, col], _F32)
                wv = jnp.where(no8, carry[0], jnp.where(no8b, carry[1], wv))
                a = wv * xr_v[0, 0:8, :]
                b = wv * xr_v[1, 0:8, :]
                for k in range(1, _KR):
                    wv = jnp.full((8, _U), ws_s[row, col + k], _F32)
                    a = a + wv * xr_v[0, k * 8:k * 8 + 8, :]
                    b = b + wv * xr_v[1, k * 8:k * 8 + 8, :]
                rs = pl.ds(pl.multiple_of(drow * 8, 8), 8)
                dst[0, rs, :] = a
                dst[1, rs, :] = b
                return a, b

            def pair(row, dst, drow, carry):
                carry = column(row, 0, dst, drow, carry)
                return column(row, _KR, dst, drow + hc, carry)

            e0 = jnp.minimum((step - 1) * _NE, len(_EXTRA) * hc - _NE)

            def extra_pair(i, carry):
                e = e0 + i
                drow = (jax.lax.shift_right_logical(e, 6) * nc
                        + jnp.bitwise_and(e, hc - 1))
                return pair(e, rt2_v, drow, carry)

            row0 = (step + (len(_EXTRA) - 1)) * hc

            def main_pair(i, carry):
                return pair(row0 + i, rt_v, i, carry)

            zero = jnp.zeros((8, _U), _F32)
            carry = jax.lax.fori_loop(0, _NE, extra_pair, (zero, zero),
                                      unroll=True)
            jax.lax.fori_loop(0, hc, main_pair, carry, unroll=True)
            r_next = [rt_v[mt // 8, pl.ds(mt % 8, nc, stride=8), :].T
                      for mt in range(nmt)]

            nq = nmt * _U // _TM
            for q in range(nq):
                sl = pl.ds(q * _TM, _TM)
                x = x_v[sl, :]
                g0 = jnp.concatenate(
                    [_dot(x[i * _U:(i + 1) * _U], w_v[step, 0, :, 0:nc])
                     for i in range(_TM // _U)], axis=0)
                g = jnp.concatenate([g0, _dot(x, w_v[step, 0, :, nc:tf])],
                                    axis=1)
                u1 = _dot(x, w_v[step, 1, :, 0:tf - nc])
                u2 = (_dot(x[:, 0:_KM], w_v[step, 1, 0:_KM, tf - nc:tf])
                      + r_v[sl, :])
                h = jnp.concatenate([_act(g[:, 0:tf - nc], u1),
                                     _act(g[:, tf - nc:tf], u2)], axis=1)
                wd = w_v[step, 2]
                if q < nq - 1:
                    acc_v[:, sl] = acc_v[:, sl] + _down(wd, h)
                    continue
                r = acc_v[:, sl]
                for kk in range(_CT):
                    wk = wd[:, kk * nc:(kk + 1) * nc]
                    if kk == _CT - 1:
                        ta, tb = r_next[0][nc - 8:], r_next[1][nc - 8:]
                        for mt in range(2, nmt, 2):
                            ta = ta + r_next[mt][nc - 8:]
                            tb = tb + r_next[mt + 1][nc - 8:]
                        t = jnp.concatenate([ta, tb], axis=0).astype(_BF16)
                        mid = jnp.where(no16, t, wk[288:304])
                        wk = jnp.concatenate([wk[:288], mid, wk[304:]], axis=0)
                    r = r + _down(wk, h[:, kk * nc:(kk + 1) * nc])
                acc_v[:, sl] = r

            for mt in range(nmt):
                r_v[mt * _U:(mt + 1) * _U, :] = r_next[mt]

        @pl.when(step == last)
        def _last():
            def proj(m, x, lo, sz):
                nfull = _CT - (1 if m == 0 else 2)
                outs = [_dot(x, w_v[last, m, :, 0:nfull * nc])]
                for ct in range(nfull, _CT):
                    if (m, ct) in _EXTRA:
                        e = _EXTRA.index((m, ct))
                        rem = jnp.concatenate(
                            [rt2_v[mt // 8,
                                   pl.ds(e * nc * 8 + mt % 8, nc, stride=8),
                                   :].T
                             for mt in range(lo // _U, (lo + sz) // _U)],
                            axis=0)
                    else:
                        rem = r_v[pl.ds(lo, sz), :]
                    outs.append(_dot(x[:, 0:_KM],
                                     w_v[last, m, 0:_KM,
                                         ct * nc:(ct + 1) * nc]) + rem)
                return jnp.concatenate(outs, axis=1)

            def finish(lo, sz, rows, h):
                for rlo, rsz in rows:
                    cs, rs = pl.ds(lo, sz), pl.ds(rlo, rsz)
                    r = acc_v[rs, cs] + _down(w_v[last, 2, rs, :], h)
                    o_v[rs, cs] = r.astype(o_v.dtype)
                    o_copy(lo, sz, rlo, rsz).start()

            pending = None
            for lo, sz, rows in _LAST:
                x = x_v[pl.ds(lo, sz), :]
                h = _act(proj(0, x, lo, sz), proj(1, x, lo, sz))
                if pending is not None:
                    finish(*pending)
                pending = (lo, sz, rows, h)
            finish(*pending)
            for lo, sz, rows in _LAST:
                for rlo, rsz in rows:
                    o_copy(lo, sz, rlo, rsz).wait()

    return kernel


@jax.jit
def pallas_standalone__geglu_ffn__prompt_kernel(
    x: jax.Array,
    w_gate: jax.Array,
    w_up: jax.Array,
    w_down: jax.Array,
):
    B, S, D = x.shape
    F = w_gate.shape[1]
    M = B * S
    nch, nmt = F // _TF, M // _U
    assert D == _D and nmt == 16 and nch * _TF == F
    nvt = len(_EXTRA) + nch - 2
    xT = x.reshape(M, D).T
    wdT = w_down.T
    outT = pl.pallas_call(
        _make_kernel(nch, nmt),
        grid=(nch,),
        in_specs=[pl.BlockSpec(memory_space=pl.ANY)] * 4,
        out_specs=pl.BlockSpec(memory_space=pl.ANY),
        out_shape=jax.ShapeDtypeStruct((D, M), x.dtype),
        scratch_shapes=[
            pltpu.VMEM((D, M), _BF16),
            pltpu.VMEM((M, D), _BF16),
            pltpu.VMEM((nch, 3, D, _TF), _BF16),
            pltpu.VMEM((M, _TF), _BF16),
            pltpu.VMEM((D, M), _F32),
            pltpu.VMEM((D, M), x.dtype),
            pltpu.VMEM((2, M, _TF), _F32),
            pltpu.VMEM((_KR, _U), _BF16),
            pltpu.VMEM((nvt, _KR, _U), _BF16),
            pltpu.VMEM((nvt * _U // 2, 2 * _KR), _F32),
            pltpu.VMEM((2, _KR * 8, _U), _F32),
            pltpu.VMEM((2, _U * 8, _U), _F32),
            pltpu.VMEM((M, _U), _F32),
            pltpu.VMEM((2, 2 * _U * 8, _U), _F32),
            pltpu.SMEM((nvt * _U // 2, 2 * _KR), _F32),
            pltpu.SemaphoreType.DMA((_NSEM,)),
            pltpu.SemaphoreType.DMA((1,)),
        ],
        compiler_params=pltpu.CompilerParams(
            dimension_semantics=("arbitrary",),
            vmem_limit_bytes=100 * 1024 * 1024),
    )(xT, w_gate, w_up, wdT)
    return outT.T.reshape(B, S, D)
```

```python
import jax
import jax.numpy as jnp
import jax.experimental.pallas as pl
import jax.experimental.pallas.tpu as pltpu

_U = 128
_D = 576
_KM, _KR = 512, 64
_CT = 3
_TF = _CT * _U
_TM = 512
_NSEM = 4
_NE = 13
_EXTRA = ((0, _CT - 1), (1, _CT - 2))

_FIRST = (
    ((("x", 0, 4, _KM, _D),),
     (("T", 0, 4, _KM, _D),)),
    ((("g", _KM, _D), ("u", _KM, _D), ("x", 4, 8, _KM, _D)),
     (("T", 4, 8, _KM, _D),
      ("PK", 0, 2, _KM, _D, True, False), ("PK", 2, 4, _KM, _D, True, False),
      ("PK", 4, 6, _KM, _D, True, False), ("PK", 6, 8, _KM, _D, True, False))),
    ((("r0",), ("x", 8, 16, _KM, _D), ("x", 0, 4, 0, 256)),
     (("T", 8, 12, _KM, _D), ("T", 12, 16, _KM, _D), ("T", 0, 4, 0, 256),
      ("XR",), ("R1", 0, 8),
      ("PK", 8, 12, _KM, _D, True, False), ("PK", 12, 16, _KM, _D, True, False),
      ("R1", 8, 16))),
    ((("g", 0, _KM), ("u", 0, _KM), ("x", 0, 4, 256, _KM), ("x", 4, 8, 0, 256),
      ("rr",)),
     (("WS",), ("T", 0, 4, 256, _KM), ("T", 4, 8, 0, 256),
      ("PK", 0, 4, 0, 256, False, False), ("PK", 0, 4, 256, _KM, False, True),
      ("PK", 4, 8, 0, 256, False, False))),
    ((("x", 4, 8, 256, _KM), ("x", 8, 16, 0, _KM), ("d", 0, _D)),
     (("T", 4, 8, 256, _KM), ("T", 8, 12, 0, _KM), ("T", 12, 16, 0, _KM),
      ("DN", 0, 4), ("PK", 4, 8, 256, _KM, False, True),
      ("PK", 8, 12, 0, _KM, False, True), ("DN", 4, 8),
      ("PK", 12, 16, 0, _KM, False, True), ("DN", 8, 12), ("DN", 12, 16))),
)

_LAST = (
    (0, 512, ((0, _D),)),
    (512, 512, ((0, _D),)),
    (1024, 512, ((0, _D),)),
    (1536, 256, ((0, _D),)),
    (1792, 128, ((0, _D),)),
    (1920, 128, ((0, 288), (288, 288))),
)

_F32, _BF16 = jnp.float32, jnp.bfloat16


def _act(g, u):
    return (jax.nn.gelu(g, approximate=True) * u).astype(_BF16)


def _dot(a, b):
    return jnp.dot(a, b, preferred_element_type=_F32)


def _down(wd_t, h):
    return jax.lax.dot_general(wd_t, h, (((1,), (1,)), ((), ())),
                               preferred_element_type=_F32)


def _make_kernel(nch, nmt):
    ng = len(_FIRST)
    tf, nc = _TF, _U
    last = nch - 1
    hc = nc // 2
    vtiles = [(m, last * tf + ct * nc) for m, ct in _EXTRA]
    vtiles += [(1, (c + 1) * tf - nc) for c in range(2, nch)]
    assert (nch - 2) * _NE >= len(_EXTRA) * hc

    def kernel(xT_hbm, wg_hbm, wu_hbm, wdT_hbm, oT_hbm,
               xT_v, x_v, w_v, h_v, acc_v, o_v, gu_v,
               wr0_v, wr_v, wf_v, xr_v, rt_v, r_v, rt2_v, ws_s, sem, sem_ws):
        w_hbm = (wg_hbm, wu_hbm, wdT_hbm)
        step = pl.program_id(0)

        def group(gi):
            s = sem.at[gi % _NSEM]
            rem = pl.ds(_KM, _KR)
            cps = []
            if gi < ng:
                for ent in _FIRST[gi][0]:
                    if ent[0] == "r0":
                        cps.append(pltpu.make_async_copy(
                            wu_hbm.at[rem, pl.ds(2 * tf - nc, nc)], wr0_v, s))
                    elif ent[0] == "rr":
                        for i, (m, col) in enumerate(vtiles):
                            cps.append(pltpu.make_async_copy(
                                w_hbm[m].at[rem, pl.ds(col, nc)],
                                wr_v.at[i], s))
                    elif ent[0] == "x":
                        _, lo, hi, klo, khi = ent
                        rs = pl.ds(klo, khi - klo)
                        cs = pl.ds(lo * _U, (hi - lo) * _U)
                        cps.append(pltpu.make_async_copy(
                            xT_hbm.at[rs, cs], xT_v.at[rs, cs], s))
                    else:
                        k = "gud".index(ent[0])
                        rs = pl.ds(ent[1], ent[2] - ent[1])
                        cps.append(pltpu.make_async_copy(
                            w_hbm[k].at[rs, pl.ds(0, tf)], w_v.at[0, k, rs], s))
            else:
                for c in (range(1, 2) if gi == ng else range(2, nch)):
                    for k in range(3):
                        cps.append(pltpu.make_async_copy(
                            w_hbm[k].at[:, pl.ds(c * tf, tf)], w_v.at[c, k], s))
            return cps

        def ws_copy():
            return pltpu.make_async_copy(wf_v, ws_s, sem_ws.at[0])

        def o_copy(lo, sz, rlo, rsz):
            rs, cs = pl.ds(rlo, rsz), pl.ds(lo, sz)
            return pltpu.make_async_copy(o_v.at[rs, cs], oT_hbm.at[rs, cs],
                                         sem.at[(ng + 2) % _NSEM])

        @pl.when(step == 0)
        def _first():
            for gi in range(_NSEM):
                for c in group(gi):
                    c.start()
            for gi, (_, ops) in enumerate(_FIRST):
                for c in group(gi):
                    c.wait()
                if gi + _NSEM <= ng + 1:
                    for c in group(gi + _NSEM):
                        c.start()
                for op in ops:
                    if op[0] == "WS":
                        for i in range(len(vtiles)):
                            wt = wr_v[i].astype(_F32).T
                            wf_v[i * hc:(i + 1) * hc, :] = jnp.concatenate(
                                [wt[:hc], wt[hc:]], axis=1)
                        ws_copy().start()
                        continue
                    if op[0] == "XR":
                        for mt in range(nmt):
                            xr_v[mt // 8, pl.ds(mt % 8, _KR, stride=8), :] = (
                                xT_v[_KM:_D, mt * _U:(mt + 1) * _U]
                                .astype(_F32))
                        continue
                    if op[0] == "R1":
                        for q in range(op[1] // 2, op[2] // 2):
                            rows = pl.ds(q * 2 * _U, 2 * _U)
                            r_v[rows, :] = _dot(x_v[rows, _KM:_D], wr0_v[...])
                        continue
                    sl = pl.ds(op[1] * _U, (op[2] - op[1]) * _U)
                    if op[0] == "T":
                        ks = pl.ds(op[3], op[4] - op[3])
                        x_v[sl, ks] = xT_v[ks, sl].T
                    elif op[0] == "DN":
                        acc_v[:, sl] = _down(w_v[0, 2], h_v[sl, :])
                    else:
                        ks = pl.ds(op[3], op[4] - op[3])
                        x = x_v[sl, ks]
                        g = _dot(x, w_v[0, 0, ks, :])
                        u = _dot(x, w_v[0, 1, ks, :])
                        if not op[5]:
                            g = g + gu_v[0, sl, :]
                            u = u + gu_v[1, sl, :]
                        if op[6]:
                            h_v[sl, :] = _act(g, u)
                        else:
                            gu_v[0, sl, :] = g
                            gu_v[1, sl, :] = u
            for c in group(ng):
                c.wait()
            ws_copy().wait()

        @pl.when(jnp.logical_and(step > 0, step < last))
        def _middle():
            @pl.when(step == 2)
            def _():
                for c in group(ng + 1):
                    c.wait()

            no8 = jnp.full((8, _U), step, jnp.int32) < 0
            no8b = jnp.full((8, _U), step, jnp.int32) < -1
            no16 = jnp.full((16, _U), step, jnp.int32) < 0

            def column(row, col, dst, drow, carry):
                xa, xb = xr_v[0, 0:_KR * 8], xr_v[1, 0:_KR * 8]
                wv = jnp.full((8, _U), ws_s[row, col], _F32)
                wv = jnp.where(no8, carry[0], jnp.where(no8b, carry[1], wv))
                a = wv * xa[0:8]
                b = wv * xb[0:8]
                for k in range(1, _KR):
                    wv = jnp.full((8, _U), ws_s[row, col + k], _F32)
                    a = a + wv * xa[k * 8:k * 8 + 8]
                    b = b + wv * xb[k * 8:k * 8 + 8]
                rs = pl.ds(pl.multiple_of(drow * 8, 8), 8)
                dst[0, rs, :] = a
                dst[1, rs, :] = b
                return a, b

            def pair(row, dst, drow, carry):
                carry = column(row, 0, dst, drow, carry)
                return column(row, _KR, dst, drow + hc, carry)

            e0 = jnp.minimum((step - 1) * _NE, len(_EXTRA) * hc - _NE)

            def extra_pair(i, carry):
                e = e0 + i
                drow = (jax.lax.shift_right_logical(e, 6) * nc
                        + jnp.bitwise_and(e, hc - 1))
                return pair(e, rt2_v, drow, carry)

            row0 = (step + (len(_EXTRA) - 1)) * hc

            def main_pair(i, carry):
                return pair(row0 + i, rt_v, i, carry)

            zero = jnp.zeros((8, _U), _F32)
            carry = jax.lax.fori_loop(0, _NE, extra_pair, (zero, zero),
                                      unroll=True)
            jax.lax.fori_loop(0, hc, main_pair, carry, unroll=True)
            r_next = [rt_v[mt // 8, pl.ds(mt % 8, nc, stride=8), :].T
                      for mt in range(nmt)]

            nq = nmt * _U // _TM
            for q in range(nq):
                sl = pl.ds(q * _TM, _TM)
                x = x_v[sl, :]
                g0 = jnp.concatenate(
                    [_dot(x[i * _U:(i + 1) * _U], w_v[step, 0, :, 0:nc])
                     for i in range(_TM // _U)], axis=0)
                g = jnp.concatenate([g0, _dot(x, w_v[step, 0, :, nc:tf])],
                                    axis=1)
                u1 = _dot(x, w_v[step, 1, :, 0:tf - nc])
                u2 = (_dot(x[:, 0:_KM], w_v[step, 1, 0:_KM, tf - nc:tf])
                      + r_v[sl, :])
                h = jnp.concatenate([_act(g[:, 0:tf - nc], u1),
                                     _act(g[:, tf - nc:tf], u2)], axis=1)
                wd = w_v[step, 2]
                if q < nq - 1:
                    acc_v[:, sl] = acc_v[:, sl] + _down(wd, h)
                    continue
                r = acc_v[:, sl]
                for kk in range(_CT):
                    wk = wd[:, kk * nc:(kk + 1) * nc]
                    if kk == _CT - 1:
                        ta, tb = r_next[0][nc - 8:], r_next[1][nc - 8:]
                        for mt in range(2, nmt, 2):
                            ta = ta + r_next[mt][nc - 8:]
                            tb = tb + r_next[mt + 1][nc - 8:]
                        t = jnp.concatenate([ta, tb], axis=0).astype(_BF16)
                        mid = jnp.where(no16, t, wk[288:304])
                        wk = jnp.concatenate([wk[:288], mid, wk[304:]], axis=0)
                    r = r + _down(wk, h[:, kk * nc:(kk + 1) * nc])
                acc_v[:, sl] = r

            for mt in range(nmt):
                r_v[mt * _U:(mt + 1) * _U, :] = r_next[mt]

        @pl.when(step == last)
        def _last():
            def proj(m, x, lo, sz):
                nfull = _CT - (1 if m == 0 else 2)
                outs = [_dot(x, w_v[last, m, :, 0:nfull * nc])]
                for ct in range(nfull, _CT):
                    if (m, ct) in _EXTRA:
                        e = _EXTRA.index((m, ct))
                        rem = jnp.concatenate(
                            [rt2_v[mt // 8,
                                   pl.ds(e * nc * 8 + mt % 8, nc, stride=8),
                                   :].T
                             for mt in range(lo // _U, (lo + sz) // _U)],
                            axis=0)
                    else:
                        rem = r_v[pl.ds(lo, sz), :]
                    outs.append(_dot(x[:, 0:_KM],
                                     w_v[last, m, 0:_KM,
                                         ct * nc:(ct + 1) * nc]) + rem)
                return jnp.concatenate(outs, axis=1)

            def finish(lo, sz, rows, h):
                for rlo, rsz in rows:
                    cs, rs = pl.ds(lo, sz), pl.ds(rlo, rsz)
                    r = acc_v[rs, cs] + _down(w_v[last, 2, rs, :], h)
                    o_v[rs, cs] = r.astype(o_v.dtype)
                    o_copy(lo, sz, rlo, rsz).start()

            pending = None
            for lo, sz, rows in _LAST:
                x = x_v[pl.ds(lo, sz), :]
                h = _act(proj(0, x, lo, sz), proj(1, x, lo, sz))
                if pending is not None:
                    finish(*pending)
                pending = (lo, sz, rows, h)
            finish(*pending)
            for lo, sz, rows in _LAST:
                for rlo, rsz in rows:
                    o_copy(lo, sz, rlo, rsz).wait()

    return kernel


@jax.jit
def pallas_standalone__geglu_ffn__prompt_kernel(
    x: jax.Array,
    w_gate: jax.Array,
    w_up: jax.Array,
    w_down: jax.Array,
):
    B, S, D = x.shape
    F = w_gate.shape[1]
    M = B * S
    nch, nmt = F // _TF, M // _U
    assert D == _D and nmt == 16 and nch * _TF == F
    nvt = len(_EXTRA) + nch - 2
    xT = x.reshape(M, D).T
    wdT = w_down.T
    outT = pl.pallas_call(
        _make_kernel(nch, nmt),
        grid=(nch,),
        in_specs=[pl.BlockSpec(memory_space=pl.ANY)] * 4,
        out_specs=pl.BlockSpec(memory_space=pl.ANY),
        out_shape=jax.ShapeDtypeStruct((D, M), x.dtype),
        scratch_shapes=[
            pltpu.VMEM((D, M), _BF16),
            pltpu.VMEM((M, D), _BF16),
            pltpu.VMEM((nch, 3, D, _TF), _BF16),
            pltpu.VMEM((M, _TF), _BF16),
            pltpu.VMEM((D, M), _F32),
            pltpu.VMEM((D, M), x.dtype),
            pltpu.VMEM((2, M, _TF), _F32),
            pltpu.VMEM((_KR, _U), _BF16),
            pltpu.VMEM((nvt, _KR, _U), _BF16),
            pltpu.VMEM((nvt * _U // 2, 2 * _KR), _F32),
            pltpu.VMEM((2, _KR * 8 + 8, _U), _F32),
            pltpu.VMEM((2, _U * 8 + 8, _U), _F32),
            pltpu.VMEM((M, _U), _F32),
            pltpu.VMEM((2, 2 * _U * 8 + 8, _U), _F32),
            pltpu.SMEM((nvt * _U // 2, 2 * _KR), _F32),
            pltpu.SemaphoreType.DMA((_NSEM,)),
            pltpu.SemaphoreType.DMA((1,)),
        ],
        compiler_params=pltpu.CompilerParams(
            dimension_semantics=("arbitrary",),
            vmem_limit_bytes=100 * 1024 * 1024),
    )(xT, w_gate, w_up, wdT)
    return outT.T.reshape(B, S, D)
```
